```python
import os as _os
_os.environ.setdefault("JAX_PLATFORMS", "cpu")
import jax
import jax.numpy as jnp

def _softmax(x, axis=-1):
    return jax.nn.softmax(x, axis=axis)
def _gelu(x):
    return jax.nn.gelu(x, approximate=True)
def _silu(x):
    return jax.nn.silu(x)
def _sigmoid(x):
    return jax.nn.sigmoid(x)
def _layernorm(x, axis=-1, eps=1e-5):
    m = jnp.mean(x, axis=axis, keepdims=True)
    v = jnp.var(x, axis=axis, keepdims=True)
    return (x - m) / jnp.sqrt(v + eps)
def _scatter_add(tgt, idx, src, axis=0):
    return tgt.at[idx].add(src)
def _segment_sum(src, seg, n):
    return jax.ops.segment_sum(src, seg, n)
class _Rng:
    def __init__(self, key):
        self._k = key
    def _next(self):
        self._k, sub = jax.random.split(self._k)
        return sub
    def normal(self, shape):
        return jax.random.normal(self._next(), shape, dtype=jnp.bfloat16)
    def randint(self, lo, hi, shape):
        return jax.random.randint(self._next(), shape, lo, hi, dtype=jnp.int32)
    def uniform(self, shape, lo=0.0, hi=1.0):
        return jax.random.uniform(self._next(), shape, jnp.bfloat16, lo, hi)
    def permutation(self, n):
        return jax.random.permutation(self._next(), n)


kernel_name = 'sequential_preLN__compressed_kv_cla__dense_activation_mish__decode'

def setup_inputs():
    _rng = _Rng(jax.random.key(int.from_bytes(__import__("os").urandom(4), "little")))
    _w = (lambda a: (lambda t: t.astype(jnp.bfloat16) if jnp.issubdtype(t.dtype, jnp.floating) else t)(jnp.asarray(a)))
    def _A_setup():
        B, H, Sq, Sk, D, M = 1, 32, 1, 8192, 128, 512
        Dc = 4 * D
        return {
            "x": _w((lambda *s: _rng.normal(s) * 0.05)(B, Sq, M)),
            "c_kv": _w((lambda *s: _rng.normal(s) * 0.8)(B, Sk, Dc)),
            "w_q": _w((lambda *s: _rng.normal(s) * 0.8)(M, H, D) * (M ** -0.5)),
            "w_uk": _w((lambda *s: _rng.normal(s) * 0.8)(Dc, H, D) * (Dc ** -0.5)),
            "w_uv": _w((lambda *s: _rng.normal(s) * 0.8)(Dc, H, D) * (Dc ** -0.5)),
            "w_o": _w((lambda *s: _rng.normal(s) * 0.8)(H, D, M) * ((H * D) ** -0.5)),
        }
    _A_in = _A_setup()

    def _B_setup():
        B, S, D, F = 1, 1, 512, 1376
        return {
            "x": _w((lambda *s: _rng.normal(s) * 0.05)(B, S, D)),
            "w1": _w((lambda *s: _rng.normal(s) * 0.2)(D, F) * (D ** -0.5)),
            "b1": _w((lambda *s: _rng.normal(s) * 0.05)(F)),
            "w2": _w((lambda *s: _rng.normal(s) * 0.05)(F, D) * (F ** -0.5)),
        }
    _B_in = _B_setup()

    return {
        "A_x": _A_in["x"],
        "A_c_kv": _A_in["c_kv"],
        "A_w_q": _A_in["w_q"],
        "A_w_uk": _A_in["w_uk"],
        "A_w_uv": _A_in["w_uv"],
        "A_w_o": _A_in["w_o"],
        "B_x": _B_in["x"],
        "B_w1": _B_in["w1"],
        "B_b1": _B_in["b1"],
        "B_w2": _B_in["w2"],
    }

def reference(A_x, A_c_kv, A_w_q, A_w_uk, A_w_uv, A_w_o, B_x, B_w1, B_b1, B_w2):
    def _A_ref(x, c_kv, w_q, w_uk, w_uv, w_o):
        B, Sq, M = x.shape[0], x.shape[1], x.shape[2]
        Sk = c_kv.shape[1]
        H, D = w_q.shape[1], w_q.shape[2]
        q = jnp.einsum("bqm,mhd->bhqd", x, w_q)
        k = jnp.einsum("bkc,chd->bhkd", c_kv, w_uk)
        v = jnp.einsum("bkc,chd->bhkd", c_kv, w_uv)
        scores = jnp.einsum("bhqd,bhkd->bhqk", q, k) * (D ** -0.5)
        off = Sk - Sq
        qi = jnp.arange(Sq)[:, None]
        kj = jnp.arange(Sk)[None, :]
        cmask = kj <= (qi + off)
        scores = jnp.where(cmask[None, None], scores, -1e9)
        p = _softmax(scores, axis=-1)
        ctx = jnp.einsum("bhqk,bhkd->bhqd", p, v)
        return jnp.einsum("bhqd,hdm->bqm", ctx, w_o)

    def _B_ref(x, w1, b1, w2):
        h = jnp.einsum("bsd,df->bsf", x, w1) + b1
        sp = jnp.log1p(jnp.exp(-jnp.abs(h))) + jnp.where(h > 0, h, jnp.zeros_like(h))
        act = h * jnp.tanh(sp)
        return jnp.einsum("bsf,fd->bsd", act, w2)

    x = A_x
    h = x + _A_ref(_layernorm(x, axis=-1), A_c_kv, A_w_q, A_w_uk, A_w_uv, A_w_o)
    h2 = h + _B_ref(_layernorm(h, axis=-1), B_w1, B_b1, B_w2)
    return h2
```

```python
import jax
import jax.numpy as jnp
import jax.experimental.pallas as pl
import jax.experimental.pallas.tpu as pltpu

W2SPLITS = (0, 1024, 1280, 1376)
G = 16
CK = 512
F32 = jnp.float32
BF16 = jnp.bfloat16
NT = (((1,), (1,)), ((), ()))
TN = (((0,), (0,)), ((), ()))


def _iota(shape, dim):
    return jax.lax.broadcasted_iota(jnp.int32, shape, dim)


def _ln(v):
    m = jnp.mean(v, axis=-1, keepdims=True)
    d = v - m
    var = jnp.mean(d * d, axis=-1, keepdims=True)
    return d / jnp.sqrt(var + 1e-5)


def _dot(a, b):
    return jnp.dot(a, b, preferred_element_type=F32)


def _dot_nt(a, b):
    return jax.lax.dot_general(a, b, NT, preferred_element_type=F32)


def _kernel(x_hbm, wq_hbm, wuk_hbm, ckv_hbm, wuv_hbm, wo_hbm, w1_hbm, b1_hbm, w2_hbm,
            o_ref,
            x_v, wq_v, wuk_v, ckv_v, wuv_v, wo_v, w1_v, b1_v, w2_v, z_v, s_v, sems):
    H, D, C, SK = 32, 128, 512, 8192
    W2S = W2SPLITS
    pairs = [(wq_hbm, wq_v), (x_hbm, x_v), (wuk_hbm, wuk_v), (ckv_hbm, ckv_v),
             (wuv_hbm, wuv_v), (wo_hbm, wo_v), (b1_hbm, b1_v), (w1_hbm, w1_v)]
    pairs += [(w2_hbm.at[pl.ds(a, b - a)], w2_v.at[pl.ds(a, b - a)]) for a, b in zip(W2S[:-1], W2S[1:])]
    cps = [pltpu.make_async_copy(s, d, sems.at[i]) for i, (s, d) in enumerate(pairs)]
    for c in cps:
        c.start()
    it = iter(cps)

    hm = (_iota((H, 128), 1) % H) == _iota((H, 128), 0)

    def masked_rows_matmul(w_ref):
        def body(g, acc):
            r0 = pl.multiple_of(g * G, G)
            zr = z_v[pl.ds(r0, G), :]
            l = jnp.concatenate([jnp.where(hm, zr[b:b + 1, :], 0.0).astype(BF16) for b in range(G)], axis=1)
            k0 = pl.multiple_of(g * G * 128, G * 128)
            return acc + _dot(l, w_ref[pl.ds(k0, G * 128), :])
        return jax.lax.fori_loop(0, 128 // G, body, jnp.zeros((H, D), F32))

    next(it).wait()
    next(it).wait()
    xf = x_v[...].astype(F32).reshape(1, C)
    xn = _ln(xf).astype(BF16)
    a_m = jnp.where((_iota((128, C), 1) // 4) == _iota((128, C), 0), xn.astype(F32), 0.0).astype(BF16)
    s_m = jnp.where((_iota((C, 128), 0) % 4) == (_iota((C, 128), 1) // 32), 1.0, 0.0).astype(BF16)
    z_v[...] = _dot(a_m, s_m)
    qb = masked_rows_matmul(wq_v).astype(BF16)

    next(it).wait()

    def uk_body(g, carry):
        k0 = pl.multiple_of(g * G * 128, G * 128)
        o_g = _dot_nt(qb, wuk_v[pl.ds(k0, G * 128), :])
        rows = [jnp.sum(jnp.where(hm, o_g[:, b * 128:(b + 1) * 128], 0.0), axis=0, keepdims=True) for b in range(G)]
        z_v[pl.ds(pl.multiple_of(g * G, G), G), :] = jnp.concatenate(rows, axis=0)
        return carry
    jax.lax.fori_loop(0, 128 // G, uk_body, 0)
    z = (z_v[...] * (D ** -0.5)).astype(BF16)
    p_m = jnp.where((_iota((C, 128), 0) // 4) == _iota((C, 128), 1), 1.0, 0.0).astype(BF16)
    g_m = (_iota((C, 128), 0) % 4) == (_iota((C, 128), 1) // 32)
    f_m = jnp.where(hm, 1.0, 0.0).astype(BF16)
    zr = jnp.where(g_m, _dot(p_m, z), 0.0).astype(BF16)
    qa = _dot_nt(f_m, zr).astype(BF16)

    next(it).wait()

    def sc_body(i, mx):
        k0 = pl.multiple_of(i * CK, CK)
        s = _dot_nt(qa, ckv_v[pl.ds(k0, CK), :])
        s_v[i] = s
        for t in range(CK // 128):
            mx = jnp.maximum(mx, s[:, t * 128:(t + 1) * 128])
        return mx
    mx = jax.lax.fori_loop(0, SK // CK, sc_body, jnp.full((H, 128), -jnp.inf, F32))
    m = jnp.max(mx, axis=1, keepdims=True)

    def pv_body(i, carry):
        acc, ls = carry
        k0 = pl.multiple_of(i * CK, CK)
        p = jnp.exp(s_v[i] - m)
        for t in range(CK // 128):
            ls = ls + p[:, t * 128:(t + 1) * 128]
        return acc + _dot(p.astype(BF16), ckv_v[pl.ds(k0, CK), :]), ls
    acc, ls = jax.lax.fori_loop(0, SK // CK, pv_body, (jnp.zeros((H, C), F32), jnp.zeros((H, 128), F32)))
    lsum = jnp.sum(ls, axis=1, keepdims=True)
    cc = (acc / lsum).astype(BF16)

    t2 = jax.lax.dot_general(cc, f_m, TN, preferred_element_type=F32)
    t2 = jnp.where(g_m, t2, 0.0).astype(BF16)
    pt_m = jnp.where((_iota((128, C), 1) // 4) == _iota((128, C), 0), 1.0, 0.0).astype(BF16)
    z_v[...] = _dot(pt_m, t2)
    next(it).wait()
    ctx = masked_rows_matmul(wuv_v)

    next(it).wait()
    rows = _iota((H, D), 0)
    G2 = 4

    def wo_body(g, o5):
        l = jnp.concatenate([jnp.where(rows == g * G2 + h, ctx, 0.0).astype(BF16) for h in range(G2)], axis=1)
        k0 = pl.multiple_of(g * G2 * 128, G2 * 128)
        return o5 + _dot(l, wo_v[pl.ds(k0, G2 * 128), :])
    o5 = jax.lax.fori_loop(0, H // G2, wo_body, jnp.zeros((H, C), F32))
    h1 = xf + jnp.sum(o5, axis=0, keepdims=True)

    hn = _ln(h1).astype(BF16)
    hn8 = jnp.broadcast_to(hn, (16, C))
    next(it).wait()
    next(it).wait()
    a = _dot_nt(hn8, w1_v[...])[0:1, :] + b1_v[...].astype(F32).reshape(1, 1376)
    sp = jnp.log1p(jnp.exp(-jnp.abs(a))) + jnp.where(a > 0, a, 0.0)
    act = (a * jnp.tanh(sp)).astype(BF16)
    act8 = jnp.broadcast_to(act, (16, 1376))
    res = h1
    a0, a1 = W2S[-2], W2S[-1]
    act_col = act[:, a0:a1].astype(F32).reshape(a1 - a0, 1)
    for k, (b0, b1_) in enumerate(zip(W2S[:-2], W2S[1:-1])):
        next(it).wait()
        f = _dot(act8[:, b0:b1_], w2_v[pl.ds(b0, b1_ - b0), :])
        z_v[0:4, :] = (res + f[0:1, :]).reshape(4, 128)
        res = z_v[0:4, :].reshape(1, C)
    next(it).wait()
    tail = jnp.sum(w2_v[pl.ds(a0, a1 - a0), :].astype(F32) * act_col, axis=0, keepdims=True)
    o_ref[...] = (res + tail).astype(o_ref.dtype).reshape(o_ref.shape)


@jax.jit
def pallas_sequential_preLN__compressed_kv_cla__dense_activation_mish__decode_kernel(A_x, A_c_kv, A_w_q, A_w_uk, A_w_uv, A_w_o, B_x, B_w1, B_b1, B_w2):
    ins = (A_x, A_w_q.reshape(16384, 128), A_w_uk.reshape(16384, 128), A_c_kv.reshape(8192, 512),
           A_w_uv.reshape(16384, 128), A_w_o.reshape(4096, 512), B_w1.T, B_b1, B_w2)
    scratch = [pltpu.VMEM(a.shape, a.dtype) for a in ins]
    scratch += [pltpu.VMEM((128, 128), F32), pltpu.VMEM((8192 // CK, 32, CK), F32),
                pltpu.SemaphoreType.DMA((8 + len(W2SPLITS) - 1,))]
    return pl.pallas_call(
        _kernel,
        out_shape=jax.ShapeDtypeStruct(A_x.shape, A_x.dtype),
        in_specs=[pl.BlockSpec(memory_space=pl.ANY)] * len(ins),
        out_specs=pl.BlockSpec(memory_space=pltpu.VMEM),
        scratch_shapes=scratch,
        compiler_params=pltpu.CompilerParams(vmem_limit_bytes=64 << 20),
    )(*ins)
```
